```python
import os as _os
_os.environ.setdefault("JAX_PLATFORMS", "cpu")
import jax
import jax.numpy as jnp

def _softmax(x, axis=-1):
    return jax.nn.softmax(x, axis=axis)
def _gelu(x):
    return jax.nn.gelu(x, approximate=True)
def _silu(x):
    return jax.nn.silu(x)
def _sigmoid(x):
    return jax.nn.sigmoid(x)
def _layernorm(x, axis=-1, eps=1e-5):
    m = jnp.mean(x, axis=axis, keepdims=True)
    v = jnp.var(x, axis=axis, keepdims=True)
    return (x - m) / jnp.sqrt(v + eps)
def _scatter_add(tgt, idx, src, axis=0):
    return tgt.at[idx].add(src)
def _segment_sum(src, seg, n):
    return jax.ops.segment_sum(src, seg, n)
class _Rng:
    def __init__(self, key):
        self._k = key
    def _next(self):
        self._k, sub = jax.random.split(self._k)
        return sub
    def normal(self, shape):
        return jax.random.normal(self._next(), shape, dtype=jnp.bfloat16)
    def randint(self, lo, hi, shape):
        return jax.random.randint(self._next(), shape, lo, hi, dtype=jnp.int32)
    def uniform(self, shape, lo=0.0, hi=1.0):
        return jax.random.uniform(self._next(), shape, jnp.bfloat16, lo, hi)
    def permutation(self, n):
        return jax.random.permutation(self._next(), n)


kernel_name = 'sequential_preLN__linear_kernel_hedgehog__geglu_ffn__prompt'

def setup_inputs():
    _rng = _Rng(jax.random.key(int.from_bytes(__import__("os").urandom(4), "little")))
    _w = (lambda a: (lambda t: t.astype(jnp.bfloat16) if jnp.issubdtype(t.dtype, jnp.floating) else t)(jnp.asarray(a)))
    def _A_setup():
        B, S, D, H = 1, 2048, 640, 32
        Dh = D // H
        return {
            "x": _w((lambda *s: _rng.normal(s) * 0.05)(B, S, D)),
            "wqkv": _w((lambda *s: _rng.normal(s) * 0.2)(D, 3 * D)),
            "w_phi": _w((lambda *s: _rng.normal(s) * 0.2)(H, Dh, Dh) * (Dh ** -0.5)),
            "wo": _w((lambda *s: _rng.normal(s) * 0.05)(D, D)),
        }
    _A_in = _A_setup()

    def _B_setup():
        B, S, D, F = 1, 2048, 640, 1536
        return {
            "x": _w((lambda *s: _rng.normal(s) * 0.05)(B, S, D)),
            "w_gate": _w((lambda *s: _rng.normal(s) * 0.05)(D, F)),
            "w_up": _w((lambda *s: _rng.normal(s) * 0.05)(D, F)),
            "w_down": _w((lambda *s: _rng.normal(s) * 0.05)(F, D)),
        }
    _B_in = _B_setup()

    return {
        "A_x": _A_in["x"],
        "A_wqkv": _A_in["wqkv"],
        "A_w_phi": _A_in["w_phi"],
        "A_wo": _A_in["wo"],
        "B_x": _B_in["x"],
        "B_w_gate": _B_in["w_gate"],
        "B_w_up": _B_in["w_up"],
        "B_w_down": _B_in["w_down"],
    }

def reference(A_x, A_wqkv, A_w_phi, A_wo, B_x, B_w_gate, B_w_up, B_w_down):
    def _A_ref(x, wqkv, w_phi, wo):
        B, S, D = x.shape
        H = 32; Dh = D // H
        qkv = (lambda x, *d: x.transpose(*d))((x @ wqkv).reshape(B, S, 3, H, Dh), 2, 0, 3, 1, 4)
        q, k, v = qkv[0], qkv[1], qkv[2]
        pq = jnp.einsum("bhsd,hdf->bhsf", q, w_phi)
        pk = jnp.einsum("bhsd,hdf->bhsf", k, w_phi)
        phi_q = jnp.concatenate([_softmax(pq, axis=-1), _softmax(-pq, axis=-1)], axis=-1)
        phi_k = jnp.concatenate([_softmax(pk, axis=-1), _softmax(-pk, axis=-1)], axis=-1)
        kv = jnp.einsum("bhsf,bhsd->bhfd", phi_k, v)
        z  = jnp.einsum("bhsf->bhf", phi_k)
        num = jnp.einsum("bhqf,bhfd->bhqd", phi_q, kv)
        den = jnp.einsum("bhqf,bhf->bhq", phi_q, z)[..., None] + 1e-6
        o = num / den
        return (lambda x, *d: x.transpose(*d))(o, 0, 2, 1, 3).reshape(B, S, D) @ wo

    def _B_ref(x, w_gate, w_up, w_down):
        return (_gelu(x @ w_gate) * (x @ w_up)) @ w_down

    x = A_x
    h = x + _A_ref(_layernorm(x, axis=-1), A_wqkv, A_w_phi, A_wo)
    h2 = h + _B_ref(_layernorm(h, axis=-1), B_w_gate, B_w_up, B_w_down)
    return h2
```

```python
import functools
import numpy as np
import jax
import jax.numpy as jnp
from jax import lax
import jax.experimental.pallas as pl
import jax.experimental.pallas.tpu as pltpu

S, D, H, DH, F = 2048, 640, 32, 20, 1536
G = 4
NG = H // G
GR = G * DH
TS = 512
NT = S // TS
F32, BF16 = jnp.float32, jnp.bfloat16
NT_DIMS = (((1,), (1,)), ((), ()))
NN_DIMS = (((1,), (0,)), ((), ()))


def _dot(a, b, dims=NN_DIMS):
    return lax.dot_general(a, b, dims, preferred_element_type=F32)


def _ln(x):
    m = jnp.mean(x, axis=-1, keepdims=True)
    c = x - m
    v = jnp.mean(c * c, axis=-1, keepdims=True)
    return c * lax.rsqrt(v + 1e-5)


def _red(op, parts):
    acc = parts[0]
    for p in parts[1:]:
        acc = op(acc, p)
    return op(acc, pltpu.roll(acc, 4, 0))


def _dual_exp(p):
    parts = [p[8 * i:8 * i + 8] for i in range(GR // 8)]
    mx = _red(jnp.maximum, parts)
    mn = _red(jnp.minimum, parts)
    ep = [jnp.exp(a - mx) for a in parts]
    en = [jnp.exp(mn - a) for a in parts]
    return ep, en, _red(jnp.add, ep), _red(jnp.add, en)


def _kernel(x_hbm, wqkv_hbm, wphi_ref, wo_hbm, wg_hbm, wu_hbm, wd_hbm, out_hbm,
            x_v, xn_v, wraw, wo_v, wg_v, wu_v, wd_v, w2_v, bd_v, wkv_t, wq_t,
            kv_acc, a_v, z_v, obuf, in_sems, out_sems):
    def x_copy(t):
        return pltpu.make_async_copy(x_hbm.at[pl.ds(t * TS, TS)], x_v.at[pl.ds(t * TS, TS)], in_sems.at[t])

    def w_copy(i):
        return pltpu.make_async_copy(wqkv_hbm.at[:, pl.ds(i * D, D)], wraw.at[i], in_sems.at[NT + i])

    big = [pltpu.make_async_copy(s, d, in_sems.at[NT + 3 + i])
           for i, (s, d) in enumerate(((wo_hbm, wo_v), (wg_hbm, wg_v), (wu_hbm, wu_v), (wd_hbm, wd_v)))]

    w_copy(1).start()
    x_copy(0).start()
    w_copy(2).start()
    for t in range(1, NT):
        x_copy(t).start()
    w_copy(0).start()
    for c in big:
        c.start()

    for h in range(H):
        w2_v[pl.ds(h * DH, DH), :] = wphi_ref[h].astype(F32)
    r = lax.broadcasted_iota(jnp.int32, (D, DH), 0)
    c = lax.broadcasted_iota(jnp.int32, (D, DH), 1)
    e_t = jnp.where((r % GR) // G == c, 1.0, 0.0).astype(BF16)
    bd = _dot(e_t, w2_v[...].astype(BF16), NT_DIMS)
    r = lax.broadcasted_iota(jnp.int32, (D, D), 0)
    c = lax.broadcasted_iota(jnp.int32, (D, D), 1)
    bd_v[...] = jnp.where((r // GR) * G + r % G == c // DH, bd, 0.0).astype(BF16)

    def fold(i, dst):
        for g in range(NG):
            lo, hi = (g * GR) // 128, (g * GR + GR - 1) // 128 + 1
            acc = _dot(bd_v[g * GR:(g + 1) * GR, lo * 128:hi * 128], wraw[i, :, lo * 128:hi * 128], NT_DIMS)
            dst[g * GR:(g + 1) * GR, :] = acc.astype(BF16)

    w_copy(1).wait()
    fold(1, wkv_t)
    w_copy(2).wait()
    wkv_t[D:2 * D, :] = wraw[2].T
    kv_acc[...] = jnp.zeros_like(kv_acc)

    def phase1(t, carry):
        rows = pl.ds(pl.multiple_of(t * TS, TS), TS)
        pltpu.make_async_copy(x_hbm.at[rows], x_v.at[rows], in_sems.at[t]).wait()
        xn = _ln(x_v[rows, :].astype(F32)).astype(BF16)
        xn_v[rows, :] = xn
        kvt = _dot(wkv_t[...], xn, NT_DIMS)
        ones = jnp.ones((16, TS), BF16)
        for g in range(NG):
            ep, en, sp, sn = _dual_exp(kvt[g * GR:(g + 1) * GR])
            rp, rn = 1.0 / sp, 1.0 / sn
            phi = jnp.concatenate([a * rp for a in ep] + [a * rn for a in en], axis=0).astype(BF16)
            vt = jnp.concatenate([kvt[D + g * GR:D + (g + 1) * GR].astype(BF16), ones], axis=0)
            kv_acc[g] += _dot(phi, vt, NT_DIMS)
        return carry

    lax.fori_loop(0, NT, phase1, 0)

    w_copy(0).wait()
    fold(0, wq_t)
    r = lax.broadcasted_iota(jnp.int32, (GR, 2 * GR), 0)
    c = lax.broadcasted_iota(jnp.int32, (GR, 2 * GR), 1)
    amask = r // DH == c % G
    for g in range(NG):
        kvf = kv_acc[g]
        z_v[g] = jnp.broadcast_to(kvf[:, GR:GR + 1], (2 * GR, 128))
        a_v[g] = jnp.where(amask, kvf.T[:GR], 0.0).astype(BF16)
    for c_ in big:
        c_.wait()

    def out_copy(t, slot):
        return pltpu.make_async_copy(obuf.at[slot], out_hbm.at[pl.ds(pl.multiple_of(t * TS, TS), TS)], out_sems.at[slot])

    def phase2(t, carry):
        rows = pl.ds(pl.multiple_of(t * TS, TS), TS)
        slot = t % 2
        pq = _dot(wq_t[...], xn_v[rows, :], NT_DIMS)
        outs = []
        for g in range(NG):
            ep, en, sp, sn = _dual_exp(pq[g * GR:(g + 1) * GR])
            z = z_v[g]
            zt = [jnp.concatenate([z[8 * i:8 * i + 8]] * (TS // 128), axis=1) for i in range(2 * GR // 8)]
            dp = _red(jnp.add, [a * b for a, b in zip(ep, zt[:10])])
            dn = _red(jnp.add, [a * b for a, b in zip(en, zt[10:])])
            rp, rn = 1.0 / sp, 1.0 / sn
            rden = 1.0 / (dp * rp + dn * rn + 1e-6)
            rp, rn = rp * rden, rn * rden
            phi = jnp.concatenate([a * rp for a in ep] + [a * rn for a in en], axis=0).astype(BF16)
            outs.append(_dot(a_v[g], phi))
        o = jnp.concatenate(outs, axis=0).T.astype(BF16)
        h = x_v[rows, :].astype(F32) + _dot(o, wo_v[...])
        hn = _ln(h).astype(BF16)
        gate = _dot(hn, wg_v[...])
        up = _dot(hn, wu_v[...])
        act = (jax.nn.gelu(gate, approximate=True) * up).astype(BF16)
        res = h + _dot(act, wd_v[...])

        @pl.when(t >= 2)
        def _():
            out_copy(t - 2, slot).wait()

        obuf[slot] = res.astype(BF16)
        out_copy(t, slot).start()
        return carry

    lax.fori_loop(0, NT, phase2, 0)
    for t in range(NT - 2, NT):
        out_copy(t, t % 2).wait()


@jax.jit
def pallas_sequential_preLN__linear_kernel_hedgehog__geglu_ffn__prompt_kernel(
    A_x, A_wqkv, A_w_phi, A_wo, B_x, B_w_gate, B_w_up, B_w_down,
):
    del B_x
    hbm = pl.BlockSpec(memory_space=pl.ANY)
    out = pl.pallas_call(
        _kernel,
        out_shape=jax.ShapeDtypeStruct((S, D), BF16),
        in_specs=[hbm, hbm, pl.BlockSpec(memory_space=pltpu.VMEM), hbm, hbm, hbm, hbm],
        out_specs=hbm,
        scratch_shapes=[
            pltpu.VMEM((S, D), BF16), pltpu.VMEM((S, D), BF16),
            pltpu.VMEM((3, D, D), BF16), pltpu.VMEM((D, D), BF16),
            pltpu.VMEM((D, F), BF16), pltpu.VMEM((D, F), BF16), pltpu.VMEM((F, D), BF16),
            pltpu.VMEM((D, DH), F32), pltpu.VMEM((D, D), BF16),
            pltpu.VMEM((2 * D, D), BF16), pltpu.VMEM((D, D), BF16),
            pltpu.VMEM((NG, 2 * GR, GR + 16), F32), pltpu.VMEM((NG, GR, 2 * GR), BF16),
            pltpu.VMEM((NG, 2 * GR, 128), F32),
            pltpu.VMEM((2, TS, D), BF16),
            pltpu.SemaphoreType.DMA((NT + 7,)), pltpu.SemaphoreType.DMA((2,)),
        ],
        compiler_params=pltpu.CompilerParams(vmem_limit_bytes=100 * 1024 * 1024),
    )(A_x.reshape(S, D), A_wqkv, A_w_phi, A_wo, B_w_gate, B_w_up, B_w_down)
    return out.reshape(1, S, D)
```

```python
import jax
import jax.numpy as jnp
from jax import lax
import jax.experimental.pallas as pl
import jax.experimental.pallas.tpu as pltpu

S, D, H, DH, F = 2048, 640, 32, 20, 1536
G = 4
NG = H // G
GR = G * DH
TS = 512
T2 = TS // 2
NT = S // TS
RC = 16
CW = 256
KH = 256
KR = D - 2 * KH
DM = D // 2
FH = F // 2
LOG2E = 1.4426950408889634
F32, BF16 = jnp.float32, jnp.bfloat16
NT_DIMS = (((1,), (1,)), ((), ()))
NN_DIMS = (((1,), (0,)), ((), ()))

ORDER_KV2 = 'pwlmlwpwlmlwpwlmlwpwlmlwpwlmlwpwlmlwpwlmlwpwlmlwpkkwkkpkkwkkpkkwkkpkkwkkpkkwkkpkkwkkpkkwkkpkkwkk'
ORDER_KV3 = 'plmllplmllplmllplmllplmllplmllplmllpmpkkwkkpkkwkkpkkwkkpkkwkkpkkwkkpkkwkkpkkwkkpkkwkk'
ORDER_HEAD = 'wmpwmpwmpwmpwmpwmpwmpwmpffffwffffwqqqqpqqpqqrpqqpqqrpqqpqqrpqqpqqrpqqpqqrpqqpqqrpqqpqqrprowoowoowoowopnnwpnnwpnnwpnnwpnnwpnnwpnnwpnnwpnnwpnnw'
ORDER_FFN = 'gggggggggggggggqqqgqqqgqqqgqqqgqqqgqqqgqrqqgqqrqgqqqrgqqqgqrqgrgrggrgrgogogogogogogogoggggggggggggggggdnndnnnndnnnnndnnnndnnnnnddd'


def _dot(a, b, dims=NN_DIMS):
    return lax.dot_general(a, b, dims, preferred_element_type=F32)


def _ln(x):
    m = jnp.mean(x, axis=-1, keepdims=True)
    c = x - m
    v = jnp.mean(c * c, axis=-1, keepdims=True)
    return c * lax.rsqrt(v + 1e-5)


def _lhs7(a11, a12, a21, a22):
    return [a11 + a22, a21 + a22, a11, a22, a11 + a12, a21 - a11, a12 - a22]


def _rhs7(b11, b12, b21, b22):
    return [b11 + b22, b11, b12 - b22, b21 - b11, b22, b11 + b12, b21 + b22]


def _out4(m):
    m1, m2, m3, m4, m5, m6, m7 = m
    return m1 + m4 - m5 + m7, m3 + m5, m2 + m4, m1 - m2 + m3 + m6


def _geglu2(g, u):
    c = 0.7978845608028654
    w = g * u
    return w + w * jnp.tanh(g * (c + (c * 0.044715) * (g * g)))


def _two_level(fn, blk):
    outer = [[fn(blk[p][q], blk[p][q + 2], blk[p + 2][q], blk[p + 2][q + 2]) for q in range(2)] for p in range(2)]
    return [op for i in range(7) for op in fn(outer[0][0][i], outer[0][1][i], outer[1][0][i], outer[1][1][i])]


def _rcp(x):
    r = pl.reciprocal(x, approx=True)
    return r * (2.0 - x * r)


def _win(g):
    return (g * GR) // 128 * 128, ((g + 1) * GR + 127) // 128 * 128


def _red(op, parts):
    acc = parts[0]
    for p in parts[1:]:
        acc = op(acc, p)
    return op(acc, pltpu.roll(acc, G, 0))


def _dual_exp(p):
    parts = [p[8 * i:8 * i + 8] for i in range(GR // 8)]
    mx = _red(jnp.maximum, parts)
    mn = _red(jnp.minimum, parts)
    ep = [jnp.exp2(a - mx) for a in parts]
    en = [jnp.exp2(mn - a) for a in parts]
    return ep, en, _red(jnp.add, ep), _red(jnp.add, en)


def _run(pattern, **gens):
    for ch in pattern:
        next(gens[ch], None)
    for g in gens.values():
        for _ in g:
            pass


class _Packed:
    def __init__(self, ref):
        self.ref, self.dtype = ref, BF16

    def _tiles(self, idx):
        idx = idx if isinstance(idx, tuple) else (idx,)
        idx = idx + (slice(None),) * (len(self.ref.shape) - 1 - len(idx))
        cols = idx[-1]
        lo, hi = (cols.start or 0) // 128, self.ref.shape[-3] if cols.stop is None else cols.stop // 128
        return [idx[:-2] + (c, idx[-2], slice(None)) for c in range(lo, hi)]

    def __getitem__(self, idx):
        words = self.ref.bitcast(jnp.uint32)
        out = []
        for i in self._tiles(idx):
            rows = i[-2] if i[-2] == slice(None) else slice((i[-2].start or 0) // 2, i[-2].stop // 2)
            out.append(pltpu.bitcast(words[i[:-2] + (rows, i[-1])], BF16))
        return jnp.concatenate(out, axis=1)

    def __setitem__(self, idx, val):
        for k, i in enumerate(self._tiles(idx)):
            self.ref[i] = val[:, 128 * k:128 * (k + 1)].astype(BF16)

    def view(self, i):
        return _Packed(self.ref.at[i])


def _packed(*shape):
    return pltpu.VMEM(shape[:-2] + (shape[-1] // 128, shape[-2], 128), BF16)


def _take(gen, n):
    for _ in range(n):
        next(gen, None)


def _first(gen, n):
    for _ in range(n):
        next(gen, None)
        yield


def _lazy(fn, *args):
    yield from fn(*args)


def _chain(*gens):
    for g in gens:
        yield from g


def _kernel(x_hbm, wqkv_hbm, wphi_hbm, wo_hbm, wg_hbm, wu_hbm, wd_hbm, out_hbm,
            x_v, wraw, wphi_v, wo_v, wg_v, wu_v, wd_v, w2_v, bd_v,
            xt_v, xr_v, sw_v, rw_v, tgu_v, rgu_v, sd_v,
            pk_v, pv_v, pq_v, kv_acc, phi_v, a_v, z_v, ot_v, h_v, hs_v, hr_v, at_v, obuf, in_sems, x0_sems, out_sems):
    xt_v, xr_v, sw_v, rw_v, tgu_v, rgu_v, sd_v, pv_v, phi_v, hs_v, hr_v, at_v, bd_v = map(
        _Packed, (xt_v, xr_v, sw_v, rw_v, tgu_v, rgu_v, sd_v, pv_v, phi_v, hs_v, hr_v, at_v, bd_v))

    def x_copy(t):
        return pltpu.make_async_copy(x_hbm.at[t * TS:(t + 1) * TS], x_v.at[t * TS:(t + 1) * TS], in_sems.at[t])

    def w_copy(i):
        return pltpu.make_async_copy(wqkv_hbm.at[:, i * D:(i + 1) * D], wraw.at[i], in_sems.at[NT + i])

    def out_copy(r, n):
        return pltpu.make_async_copy(obuf.at[r:r + n], out_hbm.at[r:r + n], out_sems.at[r // 128])

    phi_copy = pltpu.make_async_copy(wphi_hbm, wphi_v, in_sems.at[NT + 3])
    wo_copy, wg_copy, wu_copy, wd_copy = [
        pltpu.make_async_copy(s, d, in_sems.at[NT + 4 + i])
        for i, (s, d) in enumerate(((wo_hbm, wo_v), (wg_hbm, wg_v), (wu_hbm, wu_v), (wd_hbm, wd_v)))]

    def build_bd():
        eye = (lax.broadcasted_iota(jnp.int32, (H, H), 0) == lax.broadcasted_iota(jnp.int32, (H, H), 1))
        eye = jnp.where(eye, 1.0, 0.0).astype(BF16)
        for d in range(DH):
            w2_v[pl.ds(d, H, stride=DH), :] = _dot(eye, wphi_v[d], NT_DIMS)
        r = lax.broadcasted_iota(jnp.int32, (GR, DH), 0)
        c = lax.broadcasted_iota(jnp.int32, (GR, DH), 1)
        e_t = jnp.where((r >> 2) == c, 1.0, 0.0).astype(BF16)
        for g in range(NG):
            lo, hi = _win(g)
            bd = _dot(e_t, w2_v[lo:hi, :].astype(BF16), NT_DIMS)
            r = lax.broadcasted_iota(jnp.int32, (GR, hi - lo), 0)
            c = lax.broadcasted_iota(jnp.int32, (GR, hi - lo), 1)
            first = ((r & (G - 1)) + g * G) * DH - lo
            bd_v[g, :, 0:hi - lo] = jnp.where((c >= first) & (c < first + DH), bd, 0.0).astype(BF16)

    def put_lhs(i, row, top, bot):
        for r in range(0, top.shape[0], 16):
            tp, bt = top[r:r + 16].astype(F32), bot[r:r + 16].astype(F32)
            ops = _lhs7(tp[:, :KH], tp[:, KH:2 * KH], bt[:, :KH], bt[:, KH:2 * KH])
            for j in range(7):
                sw_v[i, j, row + r:row + r + 16, :] = ops[j].astype(BF16)
            rw_v[i, row + r:row + r + 16, :] = tp[:, 2 * KH:].astype(BF16)
            rw_v[i, DM + row + r:DM + row + r + 16, :] = bt[:, 2 * KH:].astype(BF16)
            yield

    def fold(i):
        def one(g):
            lo, hi = _win(g)
            return _dot(bd_v[g, :, 0:hi - lo], wraw[i, :, lo:hi], NT_DIMS) * LOG2E
        for g in range(NG // 2):
            yield from put_lhs(i, g * GR, one(g), one(g + NG // 2))

    def prep_t(i, w_ref):
        wt = w_ref[...].T
        yield
        yield from put_lhs(i, 0, wt[:DM], wt[DM:])

    def prep_gu():
        for c in range(0, FH, 128):
            wt = [[w[k:k + 128, c0 + c:c0 + c + 128].T for w in (wg_v, wu_v) for c0 in (0, FH)]
                  for k in range(0, 2 * KH, 128)]
            for r in range(0, 128, 16):
                blk = [[a[r:r + 16].astype(F32) for a in row] for row in wt]
                for i, op in enumerate(_two_level(_rhs7, blk)):
                    tgu_v[i, c + r:c + r + 16, :] = op
                for c0 in (c, FH + c):
                    rgu_v[0, r:r + 16, c0:c0 + 128] = wg_v[2 * KH + r:2 * KH + r + 16, c0:c0 + 128]
                    rgu_v[1, r:r + 16, c0:c0 + 128] = wu_v[2 * KH + r:2 * KH + r + 16, c0:c0 + 128]
                if r % 32 == 16:
                    yield

    def prep_wd():
        for j in range(FH // 128):
            cs = slice(j * 128, (j + 1) * 128)
            left, right = wd_v[cs, :].T, wd_v[FH + j * 128:FH + (j + 1) * 128, :].T
            for r in range(0, DM, 16):
                top, bot = slice(r, r + 16), slice(DM + r, DM + r + 16)
                ops = _lhs7(*[a.astype(F32) * 0.5 for a in (left[top], right[top], left[bot], right[bot])])
                for i in range(7):
                    sd_v[i, top, cs] = ops[i].astype(BF16)
                if r % 160 == 144:
                    yield

    def ln1(t):
        for j in range(T2 // RC):
            rs = slice(j * RC, (j + 1) * RC)
            top = _ln(x_v[t * TS + j * RC:t * TS + (j + 1) * RC, :].astype(F32))
            bot = _ln(x_v[t * TS + T2 + j * RC:t * TS + T2 + (j + 1) * RC, :].astype(F32))
            ops = _rhs7(top[:, :KH], bot[:, :KH], top[:, KH:2 * KH], bot[:, KH:2 * KH])
            for i in range(7):
                xt_v[t, i, rs, :] = ops[i].astype(BF16)
            xr_v[t, rs, :] = top[:, 2 * KH:].astype(BF16)
            xr_v[t, T2 + j * RC:T2 + (j + 1) * RC, :] = bot[:, 2 * KH:].astype(BF16)
            yield

    def strassen_t(i, rhs, rem, dims, put):
        def prod(j):
            return _dot(sw_v[i, j], rhs(j), dims)

        def rest(top, half):
            return _dot(rw_v[i, top:top + DM], rem(half), dims)

        m = {}
        for j in (1, 3):
            m[j] = prod(j)
            yield
        m[2] = prod(2)
        put(DM, 0, m[1] + m[3] + rest(DM, 0))
        yield
        m[4] = prod(4)
        yield
        put(0, T2, m[2] + m[4] + rest(0, 1))
        m[0] = prod(0)
        yield
        part = m[0] - m[1] + m[2] + rest(DM, 1)
        yield
        put(DM, T2, part + prod(5))
        yield
        put(0, 0, m[0] + m[3] - m[4] + rest(0, 0) + prod(6))
        yield

    def proj(i, t, dst):
        def put(r0, c0, val):
            dst[r0:r0 + DM, c0:c0 + T2] = val.astype(dst.dtype)
        return strassen_t(i, lambda j: xt_v[t, j], lambda half: xr_v[t, half * T2:(half + 1) * T2], NT_DIMS, put)

    def k_soft(t):
        for g in range(NG):
            for c in range(0, TS, 128):
                ep, en, sp, sn = _dual_exp(pk_v[t % 2, g * GR:(g + 1) * GR, c:c + 128])
                rp, rn = _rcp(sp), _rcp(sn)
                phi_v[g, :, c:c + 128] = jnp.concatenate([a * rp for a in ep] + [a * rn for a in en], axis=0).astype(BF16)
                yield

    def k_mm(t):
        ones = jnp.ones((16, TS), BF16)
        for g in range(NG):
            kv = _dot(phi_v[g], jnp.concatenate([pv_v[t % 2, g * GR:(g + 1) * GR, :], ones], axis=0), NT_DIMS)
            kv_acc[g] = kv if t == 0 else kv_acc[g] + kv
            yield

    def kv_finish():
        r = lax.broadcasted_iota(jnp.int32, (GR, 2 * GR), 0)
        c = lax.broadcasted_iota(jnp.int32, (GR, 2 * GR), 1)
        first = (c & (G - 1)) * DH
        amask = (r >= first) & (r < first + DH)
        for g in range(NG):
            kvf = kv_acc[g]
            z_v[g] = jnp.broadcast_to(kvf[:, GR:GR + 1], (2 * GR, 128))
            a_v[g] = jnp.where(amask, kvf.T[:GR], 0.0).astype(BF16)
            yield

    phi_q = {}

    def q_soft(t):
        for g in range(NG):
            phi_q[g] = []
            z = [z_v[g, 8 * i:8 * i + 8, :] for i in range(2 * GR // 8)]
            for c in range(0, TS, 128):
                ep, en, sp, sn = _dual_exp(pq_v[t, g * GR:(g + 1) * GR, c:c + 128])
                dp = _red(jnp.add, [a * b for a, b in zip(ep, z[:GR // 8])])
                dn = _red(jnp.add, [a * b for a, b in zip(en, z[GR // 8:])])
                rp, rn = _rcp(sp), _rcp(sn)
                rden = _rcp(dp * rp + dn * rn + 1e-6)
                rp, rn = rp * rden, rn * rden
                phi_q[g].append(jnp.concatenate([a * rp for a in ep] + [a * rn for a in en], axis=0).astype(BF16))
                yield

    def q_mm(t):
        for g in range(NG):
            ot_v[g * GR:(g + 1) * GR, :] = _dot(a_v[g], jnp.concatenate(phi_q[g], axis=1))
            yield

    def o_stage(t):
        ops = _rhs7(ot_v[:KH, :T2], ot_v[:KH, T2:], ot_v[KH:2 * KH, :T2], ot_v[KH:2 * KH, T2:])

        def put(r0, c0, val):
            pk_v[0, r0:r0 + DM, c0:c0 + T2] = val
        return strassen_t(3, lambda j: ops[j].astype(BF16),
                          lambda half: ot_v[2 * KH:, half * T2:(half + 1) * T2].astype(BF16), NN_DIMS, put)

    def ln2(t):
        att = []
        for r0 in range(0, TS, 128):
            att.append(pk_v[0, :, r0:r0 + 128].T)
            yield
        for r in range(0, 128, RC):
            blk = []
            for p in range(TS // 128):
                r0 = p * 128 + r
                h = x_v[t * TS + r0:t * TS + r0 + RC, :].astype(F32) + att[p][r:r + RC]
                h_v[t % 2, r0:r0 + RC, :] = h
                hn = _ln(h)
                hr_v[t % 2, r0:r0 + RC, :] = hn[:, 2 * KH:]
                blk.append([hn[:, c:c + 128] for c in range(0, 2 * KH, 128)])
                if p == 1:
                    yield
            for i, op in enumerate(_two_level(_lhs7, blk)):
                hs_v[t % 2, i, r:r + RC, :] = op
            yield

    def gate_up(t):
        for c in range(0, FH, CW):
            outer = []
            for i in range(7):
                m = []
                for j in range(7):
                    m.append(_dot(hs_v[t % 2, 7 * i + j], tgu_v[7 * i + j, c:c + CW], NT_DIMS))
                    if j in (3, 6):
                        yield
                outer.append(_out4(m))
            blk = [_out4([o[q] for o in outer]) for q in range(4)]
            act = []
            for side, c0 in enumerate((c, FH + c)):
                rg = _dot(hr_v[t % 2], rgu_v[0, :, c0:c0 + CW])
                yield
                ru = _dot(hr_v[t % 2], rgu_v[1, :, c0:c0 + CW])
                for half in range(2):
                    g = jnp.concatenate([blk[side][2 * half], blk[2 + side][2 * half]], axis=0)
                    u = jnp.concatenate([blk[side][2 * half + 1], blk[2 + side][2 * half + 1]], axis=0)
                    rows = slice(half * T2, (half + 1) * T2)
                    act.append(_geglu2(g + rg[rows], u + ru[rows]))
                if side == 0:
                    yield
            for i, a in enumerate(_rhs7(*act)):
                at_v[i, :, c:c + CW] = a
            yield

    def down(t):
        def finish(j, top, bot):
            ffn = jnp.concatenate([top, bot], axis=0).T
            obuf[t * TS + j * 128:t * TS + (j + 1) * 128, :] = (h_v[t % 2, j * 128:(j + 1) * 128, :] + ffn).astype(BF16)
            if t == NT - 1:
                out_copy(t * TS + j * 128, 128).start()
            elif j == TS // 128 - 1:
                out_copy(t * TS, TS).start()

        m = {}
        for j in (0, 1, 3, 4, 6, 2):
            m[j] = _dot(sd_v[j], at_v[j], NT_DIMS)
            yield
        top, bot = m[0] + m[3] - m[4] + m[6], m[1] + m[3]
        for j in range(T2 // 128):
            finish(j, top[:, j * 128:(j + 1) * 128], bot[:, j * 128:(j + 1) * 128])
        top, bot = m[2] + m[4], m[0] - m[1] + m[2]
        for j in range(T2 // 128):
            last = _dot(sd_v[5], at_v[5, j * 128:(j + 1) * 128], NT_DIMS)
            finish(T2 // 128 + j, top[:, j * 128:(j + 1) * 128], bot[:, j * 128:(j + 1) * 128] + last)
            yield

    def pkv(t):
        return _chain(proj(1, t, pk_v.at[t % 2]), proj(2, t, pv_v.view(t % 2)))

    first_x = [pltpu.make_async_copy(x_hbm.at[r:r + T2 // 2], x_v.at[r:r + T2 // 2], x0_sems.at[i])
               for i, r in enumerate((0, T2, T2 // 2, T2 + T2 // 2))]
    phi_copy.start()
    w_copy(1).start()
    phi_copy.wait()
    build_bd()
    for c in first_x:
        c.start()
    w_copy(2).start()
    w_copy(1).wait()
    _run('', w=fold(1))
    ln_0 = ln1(0)
    first_x[0].wait()
    first_x[1].wait()
    _take(ln_0, 8)
    first_x[2].wait()
    first_x[3].wait()
    proj_k = proj(1, 0, pk_v.at[0])
    _run('', l=ln_0)
    _take(proj_k, 3)
    w_copy(2).wait()
    for c in (x_copy(1), w_copy(0), x_copy(2), wg_copy, wu_copy, x_copy(3), wo_copy, wd_copy):
        c.start()
    _run('w' + 'pwwwww' * 4, p=proj_k, w=prep_t(2, wraw.at[2]))

    _run('pkkkk' * 8, p=proj(2, 0, pv_v.view(0)), k=k_soft(0))
    x_copy(1).wait()
    w_copy(0).wait()
    x_copy(2).wait()
    _run('wlwlm' * 8, w=fold(0), l=ln1(1), m=k_mm(0))
    _run('pll' * 8 + 'pkkkk' * 8, p=pkv(1), l=ln1(2), k=k_soft(1))
    wg_copy.wait()
    wu_copy.wait()
    x_copy(3).wait()
    wts = _chain(prep_gu(), prep_wd())
    _run(ORDER_KV2, p=pkv(2), m=k_mm(1), l=ln1(3), k=k_soft(2), w=_first(wts, 21))
    wo_copy.wait()
    wd_copy.wait()
    _run(ORDER_KV3, p=pkv(3), m=k_mm(2), l=prep_t(3, wo_v), k=k_soft(3), w=_first(wts, 8))

    _run(ORDER_HEAD, p=_chain(*[proj(0, t, pq_v.at[t]) for t in range(NT)]), m=k_mm(3), f=kv_finish(),
         q=q_soft(0), r=q_mm(0), o=_lazy(o_stage, 0), n=ln2(0), w=wts)
    for t in range(NT - 1):
        _run(ORDER_FFN, g=gate_up(t), q=q_soft(t + 1), r=q_mm(t + 1), o=_lazy(o_stage, t + 1),
             d=down(t), n=ln2(t + 1))
    _run('', g=gate_up(NT - 1), d=down(NT - 1))
    for t in range(NT):
        n = 128 if t == NT - 1 else TS
        for r in range(t * TS, (t + 1) * TS, n):
            out_copy(r, n).wait()


@jax.jit
def pallas_sequential_preLN__linear_kernel_hedgehog__geglu_ffn__prompt_kernel(
    A_x, A_wqkv, A_w_phi, A_wo, B_x, B_w_gate, B_w_up, B_w_down,
):
    del B_x
    hbm = pl.BlockSpec(memory_space=pl.ANY)
    out = pl.pallas_call(
        _kernel,
        out_shape=jax.ShapeDtypeStruct((S, D), BF16),
        in_specs=[hbm] * 7,
        out_specs=hbm,
        scratch_shapes=[
            pltpu.VMEM((S, D), BF16),
            pltpu.VMEM((3, D, D), BF16),
            pltpu.VMEM((DH, DH, H), BF16),
            pltpu.VMEM((D, D), BF16),
            pltpu.VMEM((D, F), BF16), pltpu.VMEM((D, F), BF16), pltpu.VMEM((F, D), BF16),
            pltpu.VMEM((D, DH), F32), _packed(NG, GR, 256),
            _packed(NT, 7, T2, KH), _packed(NT, TS, KR),
            _packed(4, 7, DM, KH), _packed(4, D, KR),
            _packed(49, FH, 128), _packed(2, KR, F), _packed(7, DM, FH),
            pltpu.VMEM((2, D, TS), F32), _packed(2, D, TS), pltpu.VMEM((NT, D, TS), F32),
            pltpu.VMEM((NG, 2 * GR, GR + 16), F32), _packed(NG, 2 * GR, TS), pltpu.VMEM((NG, GR, 2 * GR), BF16),
            pltpu.VMEM((NG, 2 * GR, 128), F32),
            pltpu.VMEM((D, TS), F32),
            pltpu.VMEM((2, TS, D), F32), _packed(2, 49, 128, 128), _packed(2, TS, KR),
            _packed(7, T2, FH),
            pltpu.VMEM((S, D), BF16),
            pltpu.SemaphoreType.DMA((NT + 8,)), pltpu.SemaphoreType.DMA((4,)), pltpu.SemaphoreType.DMA((S // 128,)),
        ],
        compiler_params=pltpu.CompilerParams(vmem_limit_bytes=110 * 1024 * 1024),
    )(A_x.reshape(S, D), A_wqkv, jnp.transpose(A_w_phi, (1, 2, 0)), A_wo, B_w_gate, B_w_up, B_w_down)
    return out.reshape(1, S, D)
```
